```python
import os as _os
_os.environ.setdefault("JAX_PLATFORMS", "cpu")
import jax
import jax.numpy as jnp

def _softmax(x, axis=-1):
    return jax.nn.softmax(x, axis=axis)
def _gelu(x):
    return jax.nn.gelu(x, approximate=True)
def _silu(x):
    return jax.nn.silu(x)
def _sigmoid(x):
    return jax.nn.sigmoid(x)
def _layernorm(x, axis=-1, eps=1e-5):
    m = jnp.mean(x, axis=axis, keepdims=True)
    v = jnp.var(x, axis=axis, keepdims=True)
    return (x - m) / jnp.sqrt(v + eps)
def _scatter_add(tgt, idx, src, axis=0):
    return tgt.at[idx].add(src)
def _segment_sum(src, seg, n):
    return jax.ops.segment_sum(src, seg, n)
class _Rng:
    def __init__(self, key):
        self._k = key
    def _next(self):
        self._k, sub = jax.random.split(self._k)
        return sub
    def normal(self, shape):
        return jax.random.normal(self._next(), shape, dtype=jnp.bfloat16)
    def randint(self, lo, hi, shape):
        return jax.random.randint(self._next(), shape, lo, hi, dtype=jnp.int32)
    def uniform(self, shape, lo=0.0, hi=1.0):
        return jax.random.uniform(self._next(), shape, jnp.bfloat16, lo, hi)
    def permutation(self, n):
        return jax.random.permutation(self._next(), n)


kernel_name = 'parallel_sum__mha_block_cached__dense_activation_mish__decode'

def setup_inputs():
    _rng = _Rng(jax.random.key(int.from_bytes(__import__("os").urandom(4), "little")))
    _w = (lambda a: (lambda t: t.astype(jnp.bfloat16) if jnp.issubdtype(t.dtype, jnp.floating) else t)(jnp.asarray(a)))
    def _A_setup():
        B, Sq, D = 1, 1, 448
        H, Sk, Dh = 16, 16384, 256
        return {
            "x": _w((lambda *s: _rng.normal(s) * 0.05)(B, Sq, D)),
            "k_cache": _w((lambda *s: _rng.normal(s) * 1.6)(B, H, Sk, Dh)),
            "v_cache": _w((lambda *s: _rng.normal(s) * 0.8)(B, H, Sk, Dh)),
            "wq": _w((lambda *s: _rng.normal(s) * 1.6)(D, H * Dh) * (D ** -0.5)),
            "wo": _w((lambda *s: _rng.normal(s) * 0.8)(H * Dh, D) * ((H * Dh) ** -0.5)),
        }
    _A_in = _A_setup()

    def _B_setup():
        B, S, D, F = 1, 1, 448, 1792
        return {
            "x": _w((lambda *s: _rng.normal(s) * 0.05)(B, S, D)),
            "w1": _w((lambda *s: _rng.normal(s) * 0.8)(D, F) * (D ** -0.5)),
            "b1": _w((lambda *s: _rng.normal(s) * 0.05)(F)),
            "w2": _w((lambda *s: _rng.normal(s) * 0.05)(F, D) * (F ** -0.5)),
        }
    _B_in = _B_setup()

    return {
        "A_x": _A_in["x"],
        "A_k_cache": _A_in["k_cache"],
        "A_v_cache": _A_in["v_cache"],
        "A_wq": _A_in["wq"],
        "A_wo": _A_in["wo"],
        "B_x": _B_in["x"],
        "B_w1": _B_in["w1"],
        "B_b1": _B_in["b1"],
        "B_w2": _B_in["w2"],
    }

def reference(A_x, A_k_cache, A_v_cache, A_wq, A_wo, B_x, B_w1, B_b1, B_w2):
    def _A_ref(x, k_cache, v_cache, wq, wo):
        B, Sq, D = x.shape
        H, Dh = 16, 256
        q = (lambda x, *d: x.transpose(*d))((x @ wq).reshape(B, Sq, H, Dh), 0, 2, 1, 3)
        scores = jnp.einsum("bhqd,bhkd->bhqk", q, k_cache) * (Dh ** -0.5)
        p = _softmax(scores, axis=-1)
        o = jnp.einsum("bhqk,bhkd->bhqd", p, v_cache)
        return (lambda x, *d: x.transpose(*d))(o, 0, 2, 1, 3).reshape(B, Sq, H * Dh) @ wo

    def _B_ref(x, w1, b1, w2):
        h = jnp.einsum("bsd,df->bsf", x, w1) + b1
        sp = jnp.log1p(jnp.exp(-jnp.abs(h))) + jnp.where(h > 0, h, jnp.zeros_like(h))
        act = h * jnp.tanh(sp)
        return jnp.einsum("bsf,fd->bsd", act, w2)

    x = A_x
    xn = _layernorm(x, axis=-1)
    return x + _A_ref(xn, A_k_cache, A_v_cache, A_wq, A_wo) + _B_ref(xn, B_w1, B_b1, B_w2)
```

```python
import functools
import jax
import jax.numpy as jnp
from jax import lax
from jax.experimental import pallas as pl
from jax.experimental.pallas import tpu as pltpu

bf16 = jnp.bfloat16
f32 = jnp.float32
D, H, SK, DH, F = 448, 16, 16384, 256, 1792
NT = (((1,), (1,)), ((), ()))


def make(T=128, NS=4, R=64, order="hk", inter=1, nobc=True, flags=None):
    NSTEP = SK // T
    KB = T // R
    if order == "hk":
        ORD = [(h, kb) for h in range(H) for kb in range(KB)]
    elif order == "kh":
        ORD = [(h, kb) for kb in range(KB) for h in range(H)]
    elif order == "80":
        ORD = [(2 * hh + h0, 2 * kk + k0) for kk in range(KB // 2) for hh in range(H // 2) for k0 in range(2) for h0 in range(2)]
    ND = len(ORD)

    def kern(x_hbm, k_hbm, v_hbm, wq_hbm, wo_hbm, w1_hbm, b1_hbm, w2_hbm, o_ref,
             ring, s_ref, x_v, b1_v, wq_v, wo_v, w1_v, w2_v, rsem, wsem):
        def kv_start(src, g, slot, j):
            h, kb = ORD[j]
            row = pl.multiple_of(g * T, T) + kb * R
            pltpu.make_async_copy(src.at[0, h, pl.ds(row, R)], ring.at[slot, h, pl.ds(kb * R, R)],
                                  rsem.at[slot]).start(priority=j % 2)

        def ring_wait(slot):
            pltpu.make_async_copy(ring.at[slot], ring.at[slot], rsem.at[slot]).wait()

        def wide_start(src, dst, sem, i, half):
            rows = pl.ds(pl.multiple_of(i * 8, 8), 8)
            cols = pl.ds(half * 2048, 2048)
            pltpu.make_async_copy(src.at[rows, cols], dst.at[rows, cols], sem).start(priority=half)

        cx = pltpu.make_async_copy(x_hbm, x_v, wsem.at[0])
        cb = pltpu.make_async_copy(b1_hbm, b1_v, wsem.at[1])
        cx.start()
        cb.start()

        @pl.loop(0, D // 8)
        def _(i):
            wide_start(wq_hbm, wq_v, wsem.at[2], i, 0)
            wide_start(wq_hbm, wq_v, wsem.at[2], i, 1)

        @pl.loop(0, D // 8)
        def _(i):
            rows = pl.ds(pl.multiple_of(i * 8, 8), 8)
            pltpu.make_async_copy(w1_hbm.at[rows], w1_v.at[rows], wsem.at[3]).start(priority=0)
            pltpu.make_async_copy(w2_hbm.at[rows], w2_v.at[rows], wsem.at[4]).start(priority=1)

        row = lax.broadcasted_iota(jnp.int32, (H, 128), 0)
        row2 = lax.broadcasted_iota(jnp.int32, (H, DH), 0)

        cx.wait()
        x = x_v[0].astype(f32)
        mu = jnp.mean(x, axis=-1, keepdims=True)
        xc = x - mu
        var = jnp.mean(xc * xc, axis=-1, keepdims=True)
        xn = jnp.broadcast_to(xc / jnp.sqrt(var + 1e-5), (H, D)).astype(bf16)

        pltpu.make_async_copy(wq_v, wq_v, wsem.at[2]).wait()
        q = jnp.zeros((H, DH), f32)
        for h in range(H):
            for j in range(h * ND // H, (h + 1) * ND // H):
                kv_start(k_hbm, 0, 0, j)
            qh = jnp.dot(xn, wq_v[:, h * DH:(h + 1) * DH], preferred_element_type=f32)
            q = jnp.where(row2 == h, qh, q)
        q = (q * (DH ** -0.5)).astype(bf16)

        @pl.loop(1, NS - 1)
        def _(g):
            for j in range(ND):
                kv_start(k_hbm, g, g, j)

        cb.wait()
        pltpu.make_async_copy(w1_v, w1_v, wsem.at[3]).wait()
        pltpu.make_async_copy(w2_v, w2_v, wsem.at[4]).wait()
        hid = jnp.dot(xn, w1_v[...], preferred_element_type=f32)[0:1] + b1_v[...].astype(f32).reshape(1, F)
        sp = jnp.log1p(jnp.exp(-jnp.abs(hid))) + jnp.where(hid > 0, hid, 0.0)
        act = jnp.broadcast_to(hid * jnp.tanh(sp), (H, F)).astype(bf16)
        base = x + lax.dot_general(act, w2_v[...], NT, preferred_element_type=f32)[0:1]

        def step(g, slot, enq, compute, carry):
            ring_wait(slot)
            for h in range(H):
                if h % inter == 0:
                    for j in range(h * ND // H, (h + inter) * ND // H):
                        enq(j)
                carry = compute(h, carry)
            return carry

        def k_step(g, mx, enq):
            slot = lax.rem(g, NS)
            rowT = lax.broadcasted_iota(jnp.int32, (H, T), 0)

            def compute(h, s):
                sh = lax.dot_general(q, ring[slot, h], NT, preferred_element_type=f32)
                return sh if h == 0 else jnp.where(rowT == h, sh, s)
            s = step(g, slot, enq, compute, None)
            s_ref[g] = s
            return jnp.maximum(mx, s)

        def nslot(g):
            return lax.rem(g + NS - 1, NS)

        mx = jnp.full((H, T), -jnp.inf, f32)
        mx = lax.fori_loop(0, NSTEP - (NS - 1), lambda g, mx: k_step(
            g, mx, lambda j: kv_start(k_hbm, g + NS - 1, nslot(g), j)), mx)
        mx = lax.fori_loop(NSTEP - (NS - 1), NSTEP, lambda g, mx: k_step(
            g, mx, lambda j: kv_start(v_hbm, g + NS - 1 - NSTEP, nslot(g), j)), mx)
        m = jnp.max(mx, axis=-1, keepdims=True)

        def v_step(g, carry, enq):
            l, acc = carry
            slot = lax.rem(g + NSTEP, NS)
            p = jnp.exp(s_ref[g] - m)
            pb = p.astype(bf16)

            def compute(h, o):
                oh = jnp.dot(pb, ring[slot, h], preferred_element_type=f32)
                return oh if h == 0 else jnp.where(row2 == h, oh, o)
            o = step(g, slot, enq, compute, None)
            return l + p, acc + o

        carry = (jnp.zeros((H, T), f32), jnp.zeros((H, DH), f32))
        carry = lax.fori_loop(0, NSTEP - (NS - 1), lambda g, c: v_step(
            g, c, lambda j: kv_start(v_hbm, g + NS - 1, nslot(g + NSTEP), j)), carry)

        NW = D // 8
        per = -(-NW // (NS - 1))

        def wo_enq(g, j):
            if j // 2 < per:
                i = (g - (NSTEP - (NS - 1))) * per + j // 2

                @pl.when(i < NW)
                def _():
                    wide_start(wo_hbm, wo_v, wsem.at[5 + i // 16], i, j % 2)
        assert 2 * per <= ND, (per, ND)
        carry = lax.fori_loop(NSTEP - (NS - 1), NSTEP, lambda g, c: v_step(g, c, lambda j: wo_enq(g, j)), carry)
        l, acc = carry
        o = acc / jnp.sum(l, axis=-1, keepdims=True)
        obd = jnp.concatenate([jnp.where(row2 == h, o, 0.0).astype(bf16) for h in range(H)], axis=1)
        outs = []
        for c in range(4):
            n = min(128, D - 128 * c)
            blk = wo_v.at[pl.ds(128 * c, n)]
            pltpu.make_async_copy(blk, blk, wsem.at[5 + c]).wait()
            r = lax.dot_general(obd, blk[...], NT, preferred_element_type=f32)
            res = base[:, 128 * c:128 * c + n] + jnp.sum(r, axis=0, keepdims=True)
            o_ref[0, :, 128 * c:128 * c + n] = res.astype(o_ref.dtype)

    def fn(A_x, A_k_cache, A_v_cache, A_wq, A_wo, B_x, B_w1, B_b1, B_w2):
        hbm = pl.BlockSpec(memory_space=pltpu.HBM)
        return pl.pallas_call(
            kern,
            in_specs=[hbm] * 8,
            out_specs=pl.BlockSpec(memory_space=pltpu.VMEM),
            out_shape=jax.ShapeDtypeStruct((1, 1, D), bf16),
            scratch_shapes=[
                pltpu.VMEM((NS, H, T, DH), bf16),
                pltpu.VMEM((NSTEP, H, T), f32),
                pltpu.VMEM((1, 1, D), bf16),
                pltpu.VMEM((F,), bf16),
                pltpu.VMEM((D, H * DH), bf16),
                pltpu.VMEM((D, H * DH), bf16),
                pltpu.VMEM((D, F), bf16),
                pltpu.VMEM((D, F), bf16),
                pltpu.SemaphoreType.DMA((NS,)),
                pltpu.SemaphoreType.DMA((9,)),
            ],
            compiler_params=pltpu.CompilerParams(
                vmem_limit_bytes=100 * 2**20, disable_bounds_checks=nobc, flags=flags),
        )(A_x, A_k_cache, A_v_cache, A_wq, A_wo.T, B_w1, B_b1, B_w2.T)
    return fn


_impl = make(128, 8, inter=4)


@jax.jit
def pallas_parallel_sum__mha_block_cached__dense_activation_mish__decode_kernel(
    A_x, A_k_cache, A_v_cache, A_wq, A_wo, B_x, B_w1, B_b1, B_w2):
    return _impl(A_x, A_k_cache, A_v_cache, A_wq, A_wo, B_x, B_w1, B_b1, B_w2)
```

```python
import jax
import jax.numpy as jnp
from jax import lax
import jax.experimental.pallas as pl
import jax.experimental.pallas.tpu as pltpu

D, H, SK, DH, F = 448, 16, 16384, 256, 1792

GROUPS, SEGS, SEG_LEN = 8, 16, 2048
GROUP_COLS = 2 * DH
TILE = 128
PIECE = 32
GROUP_STEPS = SEG_LEN // TILE
STEPS = GROUPS * GROUP_STEPS
STEP_COPIES = 16
SLOTS = 8
SKEW = 26

STRIP = 8
STRIPS = D // STRIP
W2_ON_QUEUE0 = 15
W2_STAGES = (0, 32, 48, 56)
MLP_COLS = 256

AT_WQ = 0
AT_WO = AT_WQ + 64
AT_W1 = AT_WO + 64
AT_K = AT_W1 + STRIPS // 2
AT_V = AT_K + STEPS * STEP_COPIES
AT_W2 = AT_V + STEPS * STEP_COPIES

SEM_X, SEM_B1, SEM_WQ, SEM_WO, SEM_W1, SEM_W2 = range(6)


def _aligned(start, size):
    if isinstance(start, int):
        return pl.ds(start, size)
    return pl.ds(pl.multiple_of(start, size), size)


def _dot(a, b):
    return jnp.dot(a, b, preferred_element_type=jnp.float32)


def _dot_t(a, b):
    return lax.dot_general(
        a, b, (((1,), (1,)), ((), ())), preferred_element_type=jnp.float32
    )


def _wait_filled(buf, sem):
    pltpu.make_async_copy(buf, buf, sem).wait()


def _kernel(
    x_hbm, k_hbm, v_hbm, wq_hbm, wo_hbm, w1_hbm, b1_hbm, w2_hbm,
    out_ref,
    ring, x_buf, b1_buf, wq_buf, wo_buf, w1_buf, w2_buf,
    bias_ref, q_ref, score_ref, max_ref, act_ref, sum_ref,
    ring_sems, sems,
):
    f32, bf16 = jnp.float32, jnp.bfloat16

    def copy_cache(cache, step, i, queue):
        segs = pl.ds(4 * (i & 3) + 2 * queue, 2)
        key = (i >> 2) * PIECE
        slot = step & (SLOTS - 1)
        pltpu.make_async_copy(
            cache.at[step >> 4, segs, _aligned((step & 15) * TILE + key, PIECE)],
            ring.at[slot, segs, _aligned(key, PIECE)],
            ring_sems.at[slot],
        ).start(priority=queue)

    def copy_wide(src, dst, sem, i, queue):
        idx = (
            pl.ds(4, 3) if queue else pl.ds(0, 4),
            _aligned((i >> 3) * STRIP, STRIP),
            _aligned((i & 7) * GROUP_COLS, GROUP_COLS),
        )
        pltpu.make_async_copy(src.at[idx], dst.at[idx], sem).start(priority=queue)

    def copy_strip(src, dst, sem, i, queue):
        rows = _aligned(i * STRIP, STRIP)
        pltpu.make_async_copy(src.at[rows], dst.at[rows], sem).start(priority=queue)

    def copy_w2(i, queue):
        stage = sum((i >= first).astype(jnp.int32) for first in W2_STAGES[1:-1])
        copy_strip(w2_hbm, w2_buf, sems.at[SEM_W2 + stage], i, queue)

    def copies(queue):
        w1_first = queue * (STRIPS // 2)
        w2_first = queue * W2_ON_QUEUE0
        w2_count = STRIPS - W2_ON_QUEUE0 if queue else W2_ON_QUEUE0
        return (
            (AT_WQ, AT_WO, lambda i: copy_wide(wq_hbm, wq_buf, sems.at[SEM_WQ], i, queue)),
            (AT_WO, AT_W1, lambda i: copy_wide(wo_hbm, wo_buf, sems.at[SEM_WO], i, queue)),
            (AT_W1, AT_K, lambda i: copy_strip(w1_hbm, w1_buf, sems.at[SEM_W1], w1_first + i, queue)),
            (AT_K, AT_V, lambda i: copy_cache(k_hbm, i >> 4, i & 15, queue)),
            (AT_V, AT_W2, lambda i: copy_cache(v_hbm, i >> 4, i & 15, queue)),
            (AT_W2, AT_W2 + w2_count, lambda i: copy_w2(w2_first + i, queue)),
        )

    def feed(pos, count, lo, hi):
        @pl.loop(0, count)
        def _(i):
            for queue in range(2):
                lead = queue * SKEW
                at = pos + i + lead
                for first, end, start in copies(queue):
                    if end <= lo + lead or hi + lead <= first:
                        continue
                    if first <= lo + lead and hi + lead <= end:
                        start(at - first)
                    else:
                        inside = jnp.logical_and(at >= first, at < end)
                        pl.when(inside)(lambda: start(at - first))

    def next_step(cache, at_cache, step):
        unrolled = STEPS - 1 - pl.cdiv(SKEW, STEP_COPIES)

        @pl.when(step < unrolled)
        def _():
            for i in range(STEP_COPIES):
                for queue in range(2):
                    later, j = divmod(i + queue * SKEW, STEP_COPIES)
                    copy_cache(cache, step + 1 + later, j, queue)

        @pl.when(step >= unrolled)
        def _():
            feed(
                at_cache + (step + 1) * STEP_COPIES, STEP_COPIES,
                at_cache + (unrolled + 1) * STEP_COPIES,
                at_cache + (STEPS + 1) * STEP_COPIES,
            )

        slot = step & (SLOTS - 1)
        _wait_filled(ring.at[slot], ring_sems.at[slot])
        return slot

    x_copy = pltpu.make_async_copy(x_hbm, x_buf, sems.at[SEM_X])
    b1_copy = pltpu.make_async_copy(b1_hbm, b1_buf, sems.at[SEM_B1])
    feed(-SKEW, SKEW, -SKEW, 0)
    x_copy.start()
    b1_copy.start()
    per_group = 4
    at_q = AT_K + STEP_COPIES - GROUPS * per_group
    cuts = (0, AT_WO - SKEW, AT_WO, AT_W1 - SKEW, at_q)
    for lo, hi in zip(cuts, cuts[1:]):
        feed(lo, hi - lo, lo, hi)

    x_copy.wait()
    x = x_buf[0].astype(f32)
    centred = x - jnp.mean(x, axis=-1, keepdims=True)
    var = jnp.mean(centred * centred, axis=-1, keepdims=True)
    xn = jnp.broadcast_to(centred / jnp.sqrt(var + 1e-5), (SEGS, D)).astype(bf16)
    sum_ref[...] = x

    row_dh = lax.broadcasted_iota(jnp.int32, (SEGS, DH), 0)
    row_tile = lax.broadcasted_iota(jnp.int32, (SEGS, TILE), 0)
    _wait_filled(wq_buf, sems.at[SEM_WQ])

    @pl.loop(0, GROUPS)
    def _(g):
        feed(at_q + per_group * g, per_group, at_q, at_q + per_group * GROUPS)
        w = wq_buf[:, :, _aligned(g * GROUP_COLS, GROUP_COLS)].reshape(D, GROUP_COLS)
        q = _dot(xn, w) * DH**-0.5
        q_ref[g] = jnp.where(row_dh < SEGS // 2, q[:, :DH], q[:, DH:]).astype(bf16)

    b1_copy.wait()
    _wait_filled(wo_buf, sems.at[SEM_WO])
    _wait_filled(w1_buf, sems.at[SEM_W1])
    bias_ref[...] = b1_buf[...].astype(f32).reshape(1, F)

    max_ref[...] = jnp.full(max_ref.shape, -jnp.inf, f32)

    @pl.loop(0, STEPS)
    def _(step):
        slot = next_step(k_hbm, AT_K, step)
        g = step >> 4
        q = q_ref[g]
        s = _dot_t(q, ring[slot, 0])
        for j in range(1, SEGS):
            s = jnp.where(row_tile == j, _dot_t(q, ring[slot, j]), s)
        score_ref[step] = s
        max_ref[g] = jnp.maximum(max_ref[g], s)

        @pl.when(step < F // MLP_COLS)
        def _():
            cols = _aligned(step * MLP_COLS, MLP_COLS)
            h = _dot(xn, w1_buf[:, cols]) + bias_ref[:, cols]
            softplus = jnp.log1p(jnp.exp(-jnp.abs(h))) + jnp.where(h > 0, h, 0.0)
            act_ref[:, cols] = (h * jnp.tanh(softplus)).astype(bf16)

    head_max = max_ref[...].reshape(H, SEGS // 2, TILE)
    head_max = jnp.max(jnp.max(head_max, axis=2, keepdims=True), axis=1, keepdims=True)
    max_ref[...] = jnp.broadcast_to(head_max, (H, SEGS // 2, TILE)).reshape(max_ref.shape)

    def value_step(step, carry):
        slot = next_step(v_hbm, AT_V, step)
        g = step >> 4
        p = jnp.exp(score_ref[step] - max_ref[g])
        p_bf16 = p.astype(bf16)
        o = _dot(p_bf16, ring[slot, 0])
        for j in range(1, SEGS):
            o = jnp.where(row_dh == j, _dot(p_bf16, ring[slot, j]), o)
        new_group = (step & 15) == 0
        denom = jnp.where(new_group, 0.0, carry[0]) + p
        numer = jnp.where(new_group, 0.0, carry[1]) + o

        @pl.when((step & 15) == 15)
        def _():
            heads = []
            for rows in (slice(0, SEGS // 2), slice(SEGS // 2, SEGS)):
                total = jnp.sum(jnp.sum(denom[rows], axis=0, keepdims=True), axis=1, keepdims=True)
                head = jnp.sum(numer[rows], axis=0, keepdims=True) / total
                heads.append(jnp.broadcast_to(head, (SEGS, DH)).astype(bf16))
            w = wo_buf[:, :, _aligned(g * GROUP_COLS, GROUP_COLS)].reshape(D, GROUP_COLS)
            sum_ref[...] += _dot_t(jnp.concatenate(heads, axis=1), w)[0:1]

        return denom, numer

    lax.fori_loop(
        0, STEPS, value_step,
        (jnp.zeros((SEGS, TILE), f32), jnp.zeros((SEGS, DH), f32)),
    )

    act = act_ref[...]
    for stage, (lo, hi) in enumerate(zip(W2_STAGES, W2_STAGES[1:])):
        w = w2_buf.at[pl.ds(lo * STRIP, (hi - lo) * STRIP)]
        _wait_filled(w, sems.at[SEM_W2 + stage])
        cols = slice(lo * STRIP, hi * STRIP)
        out = sum_ref[:, cols] + _dot_t(act, w[...])[0:1]
        out_ref[0, :, cols] = out.astype(out_ref.dtype)


@jax.jit
def pallas_parallel_sum__mha_block_cached__dense_activation_mish__decode_kernel(
    A_x: jax.Array,
    A_k_cache: jax.Array,
    A_v_cache: jax.Array,
    A_wq: jax.Array,
    A_wo: jax.Array,
    B_x: jax.Array,
    B_w1: jax.Array,
    B_b1: jax.Array,
    B_w2: jax.Array,
):
    del B_x
    f32, bf16 = jnp.float32, jnp.bfloat16
    cache_shape = (GROUPS, SEGS, SEG_LEN, DH)
    wide_shape = (D // 64, 64, H * DH)

    return pl.pallas_call(
        _kernel,
        in_specs=[pl.BlockSpec(memory_space=pltpu.HBM)] * 8,
        out_specs=pl.BlockSpec(memory_space=pltpu.VMEM),
        out_shape=jax.ShapeDtypeStruct(A_x.shape, A_x.dtype),
        scratch_shapes=[
            pltpu.VMEM((SLOTS, SEGS, TILE, DH), bf16),
            pltpu.VMEM(A_x.shape, bf16),
            pltpu.VMEM((F,), bf16),
            pltpu.VMEM(wide_shape, bf16),
            pltpu.VMEM(wide_shape, bf16),
            pltpu.VMEM((D, F), bf16),
            pltpu.VMEM((D, F), bf16),
            pltpu.VMEM((1, F), f32),
            pltpu.VMEM((GROUPS, SEGS, DH), bf16),
            pltpu.VMEM((STEPS, SEGS, TILE), f32),
            pltpu.VMEM((GROUPS, SEGS, TILE), f32),
            pltpu.VMEM((SEGS, F), bf16),
            pltpu.VMEM((1, D), f32),
            pltpu.SemaphoreType.DMA((SLOTS,)),
            pltpu.SemaphoreType.DMA((SEM_W2 + len(W2_STAGES) - 1,)),
        ],
        compiler_params=pltpu.CompilerParams(
            vmem_limit_bytes=48 * 1024 * 1024,
            disable_bounds_checks=True,
            disable_semaphore_checks=True,
        ),
    )(
        A_x,
        A_k_cache.reshape(cache_shape),
        A_v_cache.reshape(cache_shape),
        A_wq.reshape(wide_shape),
        A_wo.T.reshape(wide_shape),
        B_w1,
        B_b1,
        B_w2.T,
    )
```
